```python
import os as _os
_os.environ.setdefault("JAX_PLATFORMS", "cpu")
import jax
import jax.numpy as jnp

def _softmax(x, axis=-1):
    return jax.nn.softmax(x, axis=axis)
def _gelu(x):
    return jax.nn.gelu(x, approximate=True)
def _silu(x):
    return jax.nn.silu(x)
def _sigmoid(x):
    return jax.nn.sigmoid(x)
def _layernorm(x, axis=-1, eps=1e-5):
    m = jnp.mean(x, axis=axis, keepdims=True)
    v = jnp.var(x, axis=axis, keepdims=True)
    return (x - m) / jnp.sqrt(v + eps)
def _scatter_add(tgt, idx, src, axis=0):
    return tgt.at[idx].add(src)
def _segment_sum(src, seg, n):
    return jax.ops.segment_sum(src, seg, n)
class _Rng:
    def __init__(self, key):
        self._k = key
    def _next(self):
        self._k, sub = jax.random.split(self._k)
        return sub
    def normal(self, shape):
        return jax.random.normal(self._next(), shape, dtype=jnp.bfloat16)
    def randint(self, lo, hi, shape):
        return jax.random.randint(self._next(), shape, lo, hi, dtype=jnp.int32)
    def uniform(self, shape, lo=0.0, hi=1.0):
        return jax.random.uniform(self._next(), shape, jnp.bfloat16, lo, hi)
    def permutation(self, n):
        return jax.random.permutation(self._next(), n)


kernel_name = 'sequential_preLN__sliding_local_dilated__dense_activation_mish__prompt'

def setup_inputs():
    _rng = _Rng(jax.random.key(int.from_bytes(__import__("os").urandom(4), "little")))
    _w = (lambda a: (lambda t: t.astype(jnp.bfloat16) if jnp.issubdtype(t.dtype, jnp.floating) else t)(jnp.asarray(a)))
    def _A_setup():
        B, S, D = 1, 2048, 512
        return {
            "x": _w((lambda *s: _rng.normal(s) * 0.05)(B, S, D)),
            "wqkv": _w((lambda *s: _rng.normal(s) * 0.05)(D, 3 * D)),
            "wo": _w((lambda *s: _rng.normal(s) * 0.05)(D, D)),
        }
    _A_in = _A_setup()

    def _B_setup():
        B, S, D, F = 1, 2048, 512, 1376
        return {
            "x": _w((lambda *s: _rng.normal(s) * 0.05)(B, S, D)),
            "w1": _w((lambda *s: _rng.normal(s) * 1.6)(D, F) * (D ** -0.5)),
            "b1": _w((lambda *s: _rng.normal(s) * 0.1)(F)),
            "w2": _w((lambda *s: _rng.normal(s) * 0.1)(F, D) * (F ** -0.5)),
        }
    _B_in = _B_setup()

    return {
        "A_x": _A_in["x"],
        "A_wqkv": _A_in["wqkv"],
        "A_wo": _A_in["wo"],
        "B_x": _B_in["x"],
        "B_w1": _B_in["w1"],
        "B_b1": _B_in["b1"],
        "B_w2": _B_in["w2"],
    }

def reference(A_x, A_wqkv, A_wo, B_x, B_w1, B_b1, B_w2):
    def _A_ref(x, wqkv, wo):
        B, S, D = x.shape
        H = 32; Dh = D // H
        W, dil = 8, 2
        qkv = (lambda x, *d: x.transpose(*d))((x @ wqkv).reshape(B, S, 3, H, Dh), 2, 0, 3, 1, 4)
        q, k, v = qkv[0], qkv[1], qkv[2]
        scale = Dh ** -0.5
        pos = jnp.arange(S)
        off = jnp.arange(W) * dil
        idx = pos[:, None] - off[None, :]
        mask = idx >= 0
        idx_c = jnp.where(mask, idx, 0).reshape(-1)
        kg = k[:, :, idx_c, :].reshape(B, H, S, W, Dh)
        vg = v[:, :, idx_c, :].reshape(B, H, S, W, Dh)
        logits = jnp.einsum("bhsd,bhswd->bhsw", q, kg) * scale
        logits = jnp.where(mask[None, None, :, :], logits, -1e9)
        attn = _softmax(logits, axis=-1)
        o = jnp.einsum("bhsw,bhswd->bhsd", attn, vg)
        return (lambda x, *d: x.transpose(*d))(o, 0, 2, 1, 3).reshape(B, S, D) @ wo

    def _B_ref(x, w1, b1, w2):
        h = jnp.einsum("bsd,df->bsf", x, w1) + b1
        sp = jnp.log1p(jnp.exp(-jnp.abs(h))) + jnp.where(h > 0, h, jnp.zeros_like(h))
        act = h * jnp.tanh(sp)
        return jnp.einsum("bsf,fd->bsd", act, w2)

    x = A_x
    h = x + _A_ref(_layernorm(x, axis=-1), A_wqkv, A_wo)
    h2 = h + _B_ref(_layernorm(h, axis=-1), B_w1, B_b1, B_w2)
    return h2
```

```python
import functools

import jax
import jax.numpy as jnp
import jax.experimental.pallas as pl
import jax.experimental.pallas.tpu as pltpu

_H = 32
_DH = 16
_W = 8
_DIL = 2
_HALO = 16
_EPS = 1e-5


def _layernorm(x):
    m = jnp.mean(x, axis=-1, keepdims=True)
    xc = x - m
    v = jnp.mean(xc * xc, axis=-1, keepdims=True)
    return xc * jax.lax.rsqrt(v + _EPS)


def _kernel(x_ref, wqkv_ref, wo_ref, w1_ref, b1_ref, w2_ref, o_ref, kv_scr, *, tm, d):
    i = pl.program_id(0)

    @pl.when(i == 0)
    def _():
        kv_scr[0:_HALO, :] = jnp.zeros((_HALO, 2 * d), jnp.float32)

    x = x_ref[...].astype(jnp.bfloat16).astype(jnp.float32)
    ln1 = _layernorm(x).astype(jnp.bfloat16)
    qkv = jnp.dot(ln1, wqkv_ref[...], preferred_element_type=jnp.float32)
    q = qkv[:, :d] * (_DH ** -0.5)
    kv_scr[_HALO:_HALO + tm, :] = qkv[:, d:]

    r = jax.lax.broadcasted_iota(jnp.int32, (128, 128), 0) // _DH
    c = jax.lax.broadcasted_iota(jnp.int32, (128, 128), 1) // _DH
    bd = jnp.where(r == c, 1.0, 0.0).astype(jnp.bfloat16)

    pos = i * tm + jax.lax.broadcasted_iota(jnp.int32, (tm, d), 0)

    logits = []
    for w in range(_W):
        k_w = kv_scr[pl.ds(_HALO - _DIL * w, tm), 0:d]
        prod = (q * k_w).astype(jnp.bfloat16)
        parts = [
            jnp.dot(prod[:, j * 128:(j + 1) * 128], bd, preferred_element_type=jnp.float32)
            for j in range(d // 128)
        ]
        lw = jnp.concatenate(parts, axis=-1)
        lw = jnp.where(pos >= _DIL * w, lw, -1e9)
        logits.append(lw)
    m = logits[0]
    for w in range(1, _W):
        m = jnp.maximum(m, logits[w])
    den = None
    acc = None
    for w in range(_W):
        p = jnp.exp(logits[w] - m)
        v_w = kv_scr[pl.ds(_HALO - _DIL * w, tm), d:2 * d]
        den = p if den is None else den + p
        acc = p * v_w if acc is None else acc + p * v_w
    o = (acc / den).astype(jnp.bfloat16)

    kv_scr[0:_HALO, :] = kv_scr[tm:tm + _HALO, :]

    h = x + jnp.dot(o, wo_ref[...], preferred_element_type=jnp.float32)
    ln2 = _layernorm(h).astype(jnp.bfloat16)
    h1 = jnp.dot(ln2, w1_ref[...], preferred_element_type=jnp.float32) + b1_ref[...].astype(jnp.float32)
    u = jnp.exp(-jnp.abs(h1))
    pos_h = h1 > 0
    num = jnp.where(pos_h, 1.0 + 2.0 * u, u * u + 2.0 * u)
    den2 = num + jnp.where(pos_h, 2.0 * u * u, 2.0)
    act = (h1 * num / den2).astype(jnp.bfloat16)
    y = jnp.dot(act, w2_ref[...], preferred_element_type=jnp.float32)
    o_ref[...] = (h + y).astype(o_ref.dtype)


@jax.jit
def pallas_sequential_preLN__sliding_local_dilated__dense_activation_mish__prompt_kernel(
    A_x: jax.Array,
    A_wqkv: jax.Array,
    A_wo: jax.Array,
    B_x: jax.Array,
    B_w1: jax.Array,
    B_b1: jax.Array,
    B_w2: jax.Array,
):
    B, S, D = A_x.shape
    F = B_w1.shape[1]
    tm = 256
    assert B == 1 and S % tm == 0
    x2 = A_x.reshape(S, D)
    b1 = B_b1.reshape(1, F)

    const = lambda i: (0, 0)
    out = pl.pallas_call(
        functools.partial(_kernel, tm=tm, d=D),
        grid=(S // tm,),
        in_specs=[
            pl.BlockSpec((tm, D), lambda i: (i, 0)),
            pl.BlockSpec((D, 3 * D), const),
            pl.BlockSpec((D, D), const),
            pl.BlockSpec((D, F), const),
            pl.BlockSpec((1, F), const),
            pl.BlockSpec((F, D), const),
        ],
        out_specs=pl.BlockSpec((tm, D), lambda i: (i, 0)),
        out_shape=jax.ShapeDtypeStruct((S, D), A_x.dtype),
        scratch_shapes=[pltpu.VMEM((tm + _HALO, 2 * D), jnp.float32)],
        compiler_params=pltpu.CompilerParams(
            dimension_semantics=("arbitrary",),
            vmem_limit_bytes=96 * 1024 * 1024,
        ),
    )(x2, A_wqkv, A_wo, B_w1, b1, B_w2)
    return out.reshape(B, S, D)
```

```python
import functools
import jax
import jax.numpy as jnp
import jax.experimental.pallas as pl
import jax.experimental.pallas.tpu as pltpu

_H = 32; _DH = 16; _W = 8; _DIL = 2; _HALO = 16; _EPS = 1e-5
TM = 256
RT = 16
SCHED = "1,2,1"
LOG2E = 1.4426950408889634

def _layernorm(x):
    m = jnp.mean(x, axis=-1, keepdims=True)
    xc = x - m
    v = jnp.mean(xc * xc, axis=-1, keepdims=True)
    return xc * jax.lax.rsqrt(v + _EPS)

def _kernel(x_ref, wqkv_ref, wo_ref, w1t_ref, b1_ref, w2_ref, o_ref,
            wqkv_p, wo_p, kv_scr, q_scr, a_scr, h_scr, act_scr, *, tm, d, rt, n):
    i = pl.program_id(0)
    nj = d // 128
    n_pre, n_att, n_ln2 = [int(s) for s in SCHED.split(",")]
    assert n_pre + n_att + n_ln2 == nj

    def stage2_chunk(c):
        c0 = c * 128
        y = jnp.dot(act_scr[...], w2_ref[:, c0:c0 + 128], preferred_element_type=jnp.float32)
        o_ref[:, c0:c0 + 128] = (h_scr[:, c0:c0 + 128] + y).astype(o_ref.dtype)

    def shifted(col0, r0):
        blk = kv_scr[r0:r0 + rt + _HALO, col0:col0 + d]
        out = {}
        for s in (0, 2, 4, 6):
            rs = blk if s == 0 else pltpu.roll(blk, s, 0)
            for b in (0, 1):
                w = (s + 8 * b) // _DIL
                out[w] = rs[_HALO - 8 * b:_HALO - 8 * b + rt, :]
        return [out[w] for w in range(_W)]

    def stage1(with_stage2):
        cidx = 0
        if with_stage2:
            for _ in range(n_pre):
                stage2_chunk(cidx); cidx += 1
        x = x_ref[...].astype(jnp.float32)
        ln1 = _layernorm(x).astype(jnp.bfloat16)
        qkv = jnp.dot(ln1, wqkv_p[...], preferred_element_type=jnp.float32)
        q_scr[...] = qkv[:, :d] * (_DH ** -0.5 * LOG2E)
        kv_scr[_HALO:_HALO + tm, :] = qkv[:, d:]
        nt = tm // rt
        for t in range(nt):
            r0 = t * rt
            q_t = q_scr[r0:r0 + rt, :]
            ks = shifted(0, r0)
            logits = []
            for w in range(_W):
                pr = q_t * ks[w]
                s = pr[:, 0:128]
                for j in range(1, nj):
                    s = s + pr[:, j * 128:(j + 1) * 128]
                s = s + pltpu.roll(s, 64, 1)
                s = s + pltpu.roll(s, 32, 1)
                logits.append(s)
            if r0 < _DIL * (_W - 1):
                pos = i * tm + r0 + jax.lax.broadcasted_iota(jnp.int32, (rt, 128), 0)
                logits = [jnp.where(pos >= _DIL * w, logits[w], -1e9 * LOG2E) for w in range(_W)]
            m = logits[0]
            for w in range(1, _W):
                m = jnp.maximum(m, logits[w])
            vs = shifted(d, r0)
            den = None; acc = None
            for w in range(_W):
                p = jnp.exp2(logits[w] - m)
                den = p if den is None else den + p
                pv = [p * vs[w][:, j * 128:(j + 1) * 128] for j in range(nj)]
                acc = pv if acc is None else [a + b for a, b in zip(acc, pv)]
            inv = 1.0 / den
            for j in range(nj):
                a_scr[r0:r0 + rt, j * 128:(j + 1) * 128] = (acc[j] * inv).astype(jnp.bfloat16)
            if with_stage2 and n_att > 0 and (t + 1) % (nt // (n_att + 1)) == 0 and cidx < n_pre + n_att:
                stage2_chunk(cidx); cidx += 1
        kv_scr[0:_HALO, :] = kv_scr[tm:tm + _HALO, :]
        h = x + jnp.dot(a_scr[...], wo_p[...], preferred_element_type=jnp.float32)
        if with_stage2:
            while cidx < nj:
                stage2_chunk(cidx); cidx += 1
        h_scr[...] = h
        ln2 = _layernorm(h).astype(jnp.bfloat16)
        h1 = jax.lax.dot_general(ln2, w1t_ref[...], (((1,), (1,)), ((), ())), preferred_element_type=jnp.float32) + b1_ref[...].astype(jnp.float32)
        e = jnp.exp(jnp.minimum(h1, 20.0))
        nn = e * (e + 2.0)
        act_scr[...] = (h1 * nn / (nn + 2.0)).astype(jnp.bfloat16)

    @pl.when(i == 0)
    def _():
        ra = jax.lax.broadcasted_iota(jnp.int32, (d, d), 0)
        cb = jax.lax.broadcasted_iota(jnp.int32, (d, d), 1)
        p_mat = jnp.where(cb == (ra % _DH) * _H + ra // _DH, 1.0, 0.0).astype(jnp.bfloat16)
        pt_mat = jnp.where(ra == (cb % _DH) * _H + cb // _DH, 1.0, 0.0).astype(jnp.bfloat16)
        for s in range(3):
            wqkv_p[:, s * d:(s + 1) * d] = jnp.dot(wqkv_ref[:, s * d:(s + 1) * d], p_mat, preferred_element_type=jnp.float32).astype(jnp.bfloat16)
        wo_p[...] = jnp.dot(pt_mat, wo_ref[...], preferred_element_type=jnp.float32).astype(jnp.bfloat16)
        kv_scr[0:_HALO, :] = jnp.zeros((_HALO, 2 * d), jnp.float32)
        stage1(False)

    @pl.when(jnp.logical_and(i > 0, i < n))
    def _():
        stage1(True)

    @pl.when(i == n)
    def _():
        for c in range(nj):
            stage2_chunk(c)

@jax.jit
def pallas_sequential_preLN__sliding_local_dilated__dense_activation_mish__prompt_kernel(A_x, A_wqkv, A_wo, B_x, B_w1, B_b1, B_w2):
    B, S, D = A_x.shape
    F = B_w1.shape[1]
    tm = TM
    n = S // tm
    x2 = A_x.reshape(S, D)
    b1 = B_b1.reshape(1, F)
    const = lambda i: (0, 0)
    out = pl.pallas_call(
        functools.partial(_kernel, tm=tm, d=D, rt=RT, n=n),
        grid=(n + 1,),
        in_specs=[
            pl.BlockSpec((tm, D), lambda i: (jnp.minimum(i, n - 1), 0)),
            pl.BlockSpec((D, 3 * D), const),
            pl.BlockSpec((D, D), const),
            pl.BlockSpec((F, D), const),
            pl.BlockSpec((1, F), const),
            pl.BlockSpec((F, D), const),
        ],
        out_specs=pl.BlockSpec((tm, D), lambda i: (jnp.maximum(i - 1, 0), 0)),
        out_shape=jax.ShapeDtypeStruct((S, D), A_x.dtype),
        scratch_shapes=[pltpu.VMEM((D, 3 * D), jnp.bfloat16), pltpu.VMEM((D, D), jnp.bfloat16),
                        pltpu.VMEM((tm + _HALO, 2 * D), jnp.float32), pltpu.VMEM((tm, D), jnp.float32), pltpu.VMEM((tm, D), jnp.bfloat16),
                        pltpu.VMEM((tm, D), jnp.float32), pltpu.VMEM((tm, F), jnp.bfloat16)],
        compiler_params=pltpu.CompilerParams(dimension_semantics=("arbitrary",), vmem_limit_bytes=96 * 1024 * 1024),
    )(x2, A_wqkv, A_wo, B_w1.T, b1, B_w2)
    return out.reshape(B, S, D)
```

```python
import functools
import jax
import jax.numpy as jnp
import jax.experimental.pallas as pl
import jax.experimental.pallas.tpu as pltpu

_H = 32; _DH = 16; _W = 8; _DIL = 2; _HALO = 16; _EPS = 1e-5
TM = 256
RT = 16
ORDER = "wq|qwqqwqq|w"
LOG2E = 1.4426950408889634

def _layernorm(x):
    m = jnp.mean(x, axis=-1, keepdims=True)
    xc = x - m
    v = jnp.mean(xc * xc, axis=-1, keepdims=True)
    return xc * jax.lax.rsqrt(v + _EPS)

def _kernel(x_ref, wqkv_hbm, wo_hbm, w1t_hbm, b1_ref, w2_hbm, o_ref,
            wqkv_ref, wo_ref, w1t_ref, w2_ref, sems,
            wqkv_p, wo_p, kv_scr, q_scr, xs_scr, ln_scr, a_scr, h_scr, act_scr, *, tm, d, rt, n):
    i = pl.program_id(0)
    nj = d // 128
    slot = i % 2
    pslot = 1 - slot
    pre, mid, post = ORDER.split("|")
    QC = 256
    nq = 3 * d // QC

    def qkv_copy(s):
        return pltpu.make_async_copy(wqkv_hbm.at[:, s * d:(s + 1) * d], wqkv_ref.at[:, s * d:(s + 1) * d], sems.at[s])
    wo_copy = pltpu.make_async_copy(wo_hbm, wo_ref, sems.at[3])
    w1_copy = pltpu.make_async_copy(w1t_hbm, w1t_ref, sems.at[4])
    w2_copy = pltpu.make_async_copy(w2_hbm, w2_ref, sems.at[5])

    def c_chunk(c):
        c0 = c * 128
        y = jnp.dot(act_scr[...], w2_ref[:, c0:c0 + 128], preferred_element_type=jnp.float32)
        o_ref[:, c0:c0 + 128] = (h_scr[:, c0:c0 + 128] + y).astype(o_ref.dtype)

    def a_ln():
        x = x_ref[...].astype(jnp.float32)
        xs_scr[slot] = x
        ln_scr[...] = _layernorm(x).astype(jnp.bfloat16)

    def a_chunk(c):
        c0 = c * QC
        r = jnp.dot(ln_scr[...], wqkv_p[:, c0:c0 + QC], preferred_element_type=jnp.float32)
        if c0 < d:
            q_scr[slot, :, c0:c0 + QC] = r * (_DH ** -0.5 * LOG2E)
        else:
            kv_scr[slot, _HALO:_HALO + tm, c0 - d:c0 - d + QC] = r

    def shifted(sl, col0, r0):
        blk = kv_scr[sl, r0:r0 + rt + _HALO, col0:col0 + 128]
        out = {}
        for s in (0, 2, 4, 6):
            rs = blk if s == 0 else pltpu.roll(blk, s, 0)
            for b in (0, 1):
                w = (s + 8 * b) // _DIL
                out[w] = rs[_HALO - 8 * b:_HALO - 8 * b + rt, :]
        return [out[w] for w in range(_W)]

    def run(do_a, do_b, do_c, first_b=False):
        st = {"q": 0, "w": 0}
        def emit(ch):
            if ch == "q" and do_a:
                a_chunk(st["q"]); st["q"] += 1
            if ch == "w" and do_c:
                c_chunk(st["w"]); st["w"] += 1
        if do_a:
            a_ln()
        for ch in pre:
            emit(ch)
        if do_b:
            nt = tm // rt
            per = max(1, nt // (len(mid) + 1))
            mi = 0
            for t in range(nt):
                r0 = t * rt
                part = None
                for j in range(nj):
                    q_j = q_scr[pslot, r0:r0 + rt, j * 128:(j + 1) * 128]
                    ks = shifted(pslot, j * 128, r0)
                    pr = [q_j * ks[w] for w in range(_W)]
                    part = pr if part is None else [a + b for a, b in zip(part, pr)]
                logits = []
                for w in range(_W):
                    s = part[w]
                    s = s + pltpu.roll(s, 64, 1)
                    s = s + pltpu.roll(s, 32, 1)
                    logits.append(s)
                if r0 < _DIL * (_W - 1):
                    pos = (i - 1) * tm + r0 + jax.lax.broadcasted_iota(jnp.int32, (rt, 128), 0)
                    logits = [jnp.where(pos >= _DIL * w, logits[w], -1e9 * LOG2E) for w in range(_W)]
                m = logits[0]
                for w in range(1, _W):
                    m = jnp.maximum(m, logits[w])
                ps = [jnp.exp2(logits[w] - m) for w in range(_W)]
                den = ps[0]
                for w in range(1, _W):
                    den = den + ps[w]
                inv = 1.0 / den
                for j in range(nj):
                    vs = shifted(pslot, d + j * 128, r0)
                    acc = ps[0] * vs[0]
                    for w in range(1, _W):
                        acc = acc + ps[w] * vs[w]
                    a_scr[r0:r0 + rt, j * 128:(j + 1) * 128] = (acc * inv).astype(jnp.bfloat16)
                if (t + 1) % per == 0 and mi < len(mid):
                    emit(mid[mi]); mi += 1
            while mi < len(mid):
                emit(mid[mi]); mi += 1
            h = xs_scr[pslot] + jnp.dot(a_scr[...], wo_p[...], preferred_element_type=jnp.float32)
        else:
            for ch in mid:
                emit(ch)
        for ch in post:
            emit(ch)
        if do_a:
            kv_scr[slot, 0:_HALO, :] = kv_scr[pslot, tm:tm + _HALO, :]
        if do_b:
            h_scr[...] = h
            ln2 = _layernorm(h).astype(jnp.bfloat16)
            if first_b:
                w1_copy.wait()
            h1 = jax.lax.dot_general(ln2, w1t_ref[...], (((1,), (1,)), ((), ())), preferred_element_type=jnp.float32) + b1_ref[...].astype(jnp.float32)
            e = jnp.exp(jnp.minimum(h1, 20.0))
            nn = e * (e + 2.0)
            act_scr[...] = (h1 * nn / (nn + 2.0)).astype(jnp.bfloat16)

    @pl.when(i == 0)
    def _():
        for s in range(3):
            qkv_copy(s).start()
        wo_copy.start()
        w1_copy.start()
        w2_copy.start()
        ra = jax.lax.broadcasted_iota(jnp.int32, (d, d), 0)
        cb = jax.lax.broadcasted_iota(jnp.int32, (d, d), 1)
        p_mat = jnp.where(cb == (ra % _DH) * _H + ra // _DH, 1.0, 0.0).astype(jnp.bfloat16)
        pt_mat = jnp.where(ra == (cb % _DH) * _H + cb // _DH, 1.0, 0.0).astype(jnp.bfloat16)
        for s in range(3):
            qkv_copy(s).wait()
            wqkv_p[:, s * d:(s + 1) * d] = jnp.dot(wqkv_ref[:, s * d:(s + 1) * d], p_mat, preferred_element_type=jnp.float32).astype(jnp.bfloat16)
        wo_copy.wait()
        wo_p[...] = jnp.dot(pt_mat, wo_ref[...], preferred_element_type=jnp.float32).astype(jnp.bfloat16)
        kv_scr[1, tm:tm + _HALO, :] = jnp.zeros((_HALO, 2 * d), jnp.float32)
        run(True, False, False)

    @pl.when(i == 1)
    def _():
        run(True, True, False, first_b=True)
        w2_copy.wait()

    @pl.when(jnp.logical_and(i > 1, i < n))
    def _():
        run(True, True, True)

    @pl.when(i == n)
    def _():
        run(False, True, True)

    @pl.when(i == n + 1)
    def _():
        run(False, False, True)

@jax.jit
def pallas_sequential_preLN__sliding_local_dilated__dense_activation_mish__prompt_kernel(A_x, A_wqkv, A_wo, B_x, B_w1, B_b1, B_w2):
    B, S, D = A_x.shape
    assert B == 1 and S % TM == 0 and S // TM >= 2 and D == _H * _DH
    F = B_w1.shape[1]
    tm = TM
    n = S // tm
    x2 = A_x.reshape(S, D)
    b1 = B_b1.reshape(1, F)
    const = lambda i: (0, 0)
    out = pl.pallas_call(
        functools.partial(_kernel, tm=tm, d=D, rt=RT, n=n),
        grid=(n + 2,),
        in_specs=[
            pl.BlockSpec((tm, D), lambda i: (jnp.minimum(i, n - 1), 0)),
            pl.BlockSpec(memory_space=pl.ANY),
            pl.BlockSpec(memory_space=pl.ANY),
            pl.BlockSpec(memory_space=pl.ANY),
            pl.BlockSpec((1, F), const),
            pl.BlockSpec(memory_space=pl.ANY),
        ],
        out_specs=pl.BlockSpec((tm, D), lambda i: (jnp.maximum(i - 2, 0), 0)),
        out_shape=jax.ShapeDtypeStruct((S, D), A_x.dtype),
        scratch_shapes=[pltpu.VMEM((D, 3 * D), jnp.bfloat16), pltpu.VMEM((D, D), jnp.bfloat16),
                        pltpu.VMEM((F, D), jnp.bfloat16), pltpu.VMEM((F, D), jnp.bfloat16),
                        pltpu.SemaphoreType.DMA((6,)),
                        pltpu.VMEM((D, 3 * D), jnp.bfloat16), pltpu.VMEM((D, D), jnp.bfloat16),
                        pltpu.VMEM((2, tm + _HALO, 2 * D), jnp.float32), pltpu.VMEM((2, tm, D), jnp.float32),
                        pltpu.VMEM((2, tm, D), jnp.float32), pltpu.VMEM((tm, D), jnp.bfloat16),
                        pltpu.VMEM((tm, D), jnp.bfloat16),
                        pltpu.VMEM((tm, D), jnp.float32), pltpu.VMEM((tm, F), jnp.bfloat16)],
        compiler_params=pltpu.CompilerParams(dimension_semantics=("arbitrary",), vmem_limit_bytes=96 * 1024 * 1024),
    )(x2, A_wqkv, A_wo, B_w1.T, b1, B_w2)
    return out.reshape(B, S, D)
```
